```python
import jax
import jax.numpy as jnp

def _softmax(x, axis=-1):
    return jax.nn.softmax(x, axis=axis)
def _gelu(x):
    return jax.nn.gelu(x, approximate=True)
def _silu(x):
    return jax.nn.silu(x)
def _sigmoid(x):
    return jax.nn.sigmoid(x)
def _layernorm(x, axis=-1, eps=1e-5):
    m = jnp.mean(x, axis=axis, keepdims=True)
    v = jnp.var(x, axis=axis, keepdims=True)
    return (x - m) / jnp.sqrt(v + eps)
def _scatter_add(tgt, idx, src, axis=0):
    return tgt.at[idx].add(src)
def _segment_sum(src, seg, n):
    return jax.ops.segment_sum(src, seg, n)
class _Rng:
    def __init__(self, key):
        self._k = key
    def _next(self):
        self._k, sub = jax.random.split(self._k)
        return sub
    def normal(self, shape):
        return jax.random.normal(self._next(), shape, dtype=jnp.bfloat16)
    def randint(self, lo, hi, shape):
        return jax.random.randint(self._next(), shape, lo, hi, dtype=jnp.int32)
    def uniform(self, shape, lo=0.0, hi=1.0):
        return jax.random.uniform(self._next(), shape, jnp.bfloat16, lo, hi)
    def permutation(self, n):
        return jax.random.permutation(self._next(), n)


kernel_name = 'gated_mix__sliding_local_dilated__compressed_kv_cla__prompt'

def setup_inputs():
    _rng = _Rng(jax.random.key(int.from_bytes(__import__("os").urandom(4), "little")))
    _w = (lambda a: (lambda t: t.astype(jnp.bfloat16) if jnp.issubdtype(t.dtype, jnp.floating) else t)(jnp.asarray(a)))
    def _A_setup():
        B, S, D = 1, 2048, 576
        return {
            "x": _w((lambda *s: _rng.normal(s) * 0.05)(B, S, D)),
            "wqkv": _w((lambda *s: _rng.normal(s) * 0.05)(D, 3 * D)),
            "wo": _w((lambda *s: _rng.normal(s) * 0.05)(D, D)),
        }
    _A_in = _A_setup()

    def _B_setup():
        B, H, Sq, Sk, D, M = 1, 32, 2048, 2048, 128, 576
        Dc = 4 * D
        return {
            "x": _w((lambda *s: _rng.normal(s) * 0.05)(B, Sq, M)),
            "c_kv": _w((lambda *s: _rng.normal(s) * 0.05)(B, Sk, Dc)),
            "w_q": _w((lambda *s: _rng.normal(s) * 0.05)(M, H, D) * (M ** -0.5)),
            "w_uk": _w((lambda *s: _rng.normal(s) * 0.05)(Dc, H, D) * (Dc ** -0.5)),
            "w_uv": _w((lambda *s: _rng.normal(s) * 0.05)(Dc, H, D) * (Dc ** -0.5)),
            "w_o": _w((lambda *s: _rng.normal(s) * 0.05)(H, D, M) * ((H * D) ** -0.5)),
        }
    _B_in = _B_setup()

    return {
        "A_x": _A_in["x"],
        "A_wqkv": _A_in["wqkv"],
        "A_wo": _A_in["wo"],
        "B_x": _B_in["x"],
        "B_c_kv": _B_in["c_kv"],
        "B_w_q": _B_in["w_q"],
        "B_w_uk": _B_in["w_uk"],
        "B_w_uv": _B_in["w_uv"],
        "B_w_o": _B_in["w_o"],
        "gate_w": _w((lambda *s: _rng.normal(s) * 0.05)(576)),
    }

def reference(A_x, A_wqkv, A_wo, B_x, B_c_kv, B_w_q, B_w_uk, B_w_uv, B_w_o, gate_w):
    def _A_ref(x, wqkv, wo):
        B, S, D = x.shape
        H = 32; Dh = D // H
        W, dil = 8, 2
        qkv = (lambda x, *d: x.transpose(*d))((x @ wqkv).reshape(B, S, 3, H, Dh), 2, 0, 3, 1, 4)
        q, k, v = qkv[0], qkv[1], qkv[2]
        scale = Dh ** -0.5
        pos = jnp.arange(S)
        off = jnp.arange(W) * dil
        idx = pos[:, None] - off[None, :]
        mask = idx >= 0
        idx_c = jnp.where(mask, idx, 0).reshape(-1)
        kg = k[:, :, idx_c, :].reshape(B, H, S, W, Dh)
        vg = v[:, :, idx_c, :].reshape(B, H, S, W, Dh)
        logits = jnp.einsum("bhsd,bhswd->bhsw", q, kg) * scale
        logits = jnp.where(mask[None, None, :, :], logits, -1e9)
        attn = _softmax(logits, axis=-1)
        o = jnp.einsum("bhsw,bhswd->bhsd", attn, vg)
        return (lambda x, *d: x.transpose(*d))(o, 0, 2, 1, 3).reshape(B, S, D) @ wo

    def _B_ref(x, c_kv, w_q, w_uk, w_uv, w_o):
        B, Sq, M = x.shape[0], x.shape[1], x.shape[2]
        Sk = c_kv.shape[1]
        H, D = w_q.shape[1], w_q.shape[2]
        q = jnp.einsum("bqm,mhd->bhqd", x, w_q)
        k = jnp.einsum("bkc,chd->bhkd", c_kv, w_uk)
        v = jnp.einsum("bkc,chd->bhkd", c_kv, w_uv)
        scores = jnp.einsum("bhqd,bhkd->bhqk", q, k) * (D ** -0.5)
        off = Sk - Sq
        qi = jnp.arange(Sq)[:, None]
        kj = jnp.arange(Sk)[None, :]
        cmask = kj <= (qi + off)
        scores = jnp.where(cmask[None, None], scores, -1e9)
        p = _softmax(scores, axis=-1)
        ctx = jnp.einsum("bhqk,bhkd->bhqd", p, v)
        return jnp.einsum("bhqd,hdm->bqm", ctx, w_o)

    x = A_x
    g = _sigmoid((x * gate_w).sum(-1, keepdims=True))
    a = _A_ref(x, A_wqkv, A_wo)
    b = _B_ref(x, B_c_kv, B_w_q, B_w_uk, B_w_uv, B_w_o)
    return g * a + (1 - g) * b
```

```python
import functools

import jax
import jax.numpy as jnp
import numpy as np
import jax.experimental.pallas as pl
import jax.experimental.pallas.tpu as pltpu

LOG2E = 1.4426950408889634
NT = (((1,), (1,)), ((), ()))
G = 4
BQ = 256
BA = 256


def _dot(a, b):
    return jnp.dot(a, b, preferred_element_type=jnp.float32)


def _kernel(x_ref, wqkv_ref, woa_ref, c_ref, wq_ref, wk_ref, wv_ref, wo_ref, gw_ref,
            o_ref, q_s, k_s, v_s, ctx_s, acc_s, a_qkv, a_out, w3, *, HA, W, DIL):
    g = pl.program_id(0)
    ng = pl.num_programs(0)
    S, M = x_ref.shape
    D = q_s.shape[-1]
    DH = M // HA
    bf = jnp.bfloat16
    PAD = a_qkv.shape[1] - S

    @pl.when(g == 0)
    def _():
        a_qkv[:, :PAD, :] = jnp.zeros((3, PAD, M), jnp.float32)

        for t in range(3):
            w3[t] = wqkv_ref[:, t * M:(t + 1) * M]

        def proj(i, carry):
            r = pl.multiple_of(i * BA, BA)
            xb = x_ref[pl.ds(r, BA), :]
            for t in range(3):
                a_qkv[t, pl.ds(PAD + r, BA), :] = _dot(xb, w3[t]).astype(bf).astype(jnp.float32)
            return carry
        jax.lax.fori_loop(0, S // BA, proj, 0)

        li = jax.lax.broadcasted_iota(jnp.int32, (M, 128), 0)
        hi = jax.lax.broadcasted_iota(jnp.int32, (M, 128), 1)
        seg = ((li >= hi * DH) & (li < hi * DH + DH)).astype(bf)
        li = jax.lax.broadcasted_iota(jnp.int32, (128, M), 1)
        hi = jax.lax.broadcasted_iota(jnp.int32, (128, M), 0)
        segt = ((li >= hi * DH) & (li < hi * DH + DH)).astype(bf)

        def loc(i, carry):
            r = pl.multiple_of(i * BA, BA)
            q = a_qkv[0, pl.ds(PAD + r, BA), :]
            pos = r + jax.lax.broadcasted_iota(jnp.int32, (BA, 128), 0)
            ls = []
            kk = a_qkv[1, pl.ds(r, BA + PAD), :]
            vv = a_qkv[2, pl.ds(r, BA + PAD), :]
            for w in range(W):
                kw = kk[PAD - w * DIL:PAD - w * DIL + BA]
                l = _dot((q * kw).astype(bf), seg) * (DH ** -0.5)
                if w:
                    l = jnp.where(pos >= w * DIL, l, -1e9)
                ls.append(l)
            m = functools.reduce(jnp.maximum, ls)
            es = [jnp.exp(l - m) for l in ls]
            inv = 1.0 / functools.reduce(jnp.add, es)
            o = None
            for w in range(W):
                vw = vv[PAD - w * DIL:PAD - w * DIL + BA]
                t = _dot((es[w] * inv).astype(bf), segt) * vw
                o = t if o is None else o + t
            a_out[pl.ds(r, BA), :] = _dot(o.astype(bf), woa_ref[...])
            return carry
        jax.lax.fori_loop(0, S // BA, loc, 0)

    def proj_b(i, carry):
        r = pl.multiple_of(i * 512, 512)
        q = _dot(x_ref[pl.ds(r, 512), :], wq_ref[...]) * (D ** -0.5 * LOG2E)
        cb = c_ref[pl.ds(r, 512), :]
        k = _dot(cb, wk_ref[...])
        v = _dot(cb, wv_ref[...])
        for h in range(G):
            q_s[h, pl.ds(r, 512), :] = q[:, h * D:(h + 1) * D].astype(bf)
            k_s[h, pl.ds(r, 512), :] = k[:, h * D:(h + 1) * D].astype(bf)
            v_s[h, pl.ds(r, 512), :] = v[:, h * D:(h + 1) * D].astype(bf)
        return carry
    jax.lax.fori_loop(0, S // 512, proj_b, 0)

    def head(h, carry):
        row = jax.lax.broadcasted_iota(jnp.int32, (BQ, BQ), 0)
        col = jax.lax.broadcasted_iota(jnp.int32, (BQ, BQ), 1)
        for i in range(S // BQ):
            lo, hi_ = i * BQ, (i + 1) * BQ
            q = q_s[h, lo:hi_, :]
            sd = jax.lax.dot_general(q, k_s[h, lo:hi_, :], NT, preferred_element_type=jnp.float32)
            sd = jnp.where(col <= row, sd, -1e9 * LOG2E)
            m = jnp.max(sd, axis=1, keepdims=True)
            if i:
                so = jax.lax.dot_general(q, k_s[h, :lo, :], NT, preferred_element_type=jnp.float32)
                m = jnp.maximum(m, jnp.max(so, axis=1, keepdims=True))
            pd = jnp.exp2(sd - m)
            l = jnp.sum(pd, axis=1, keepdims=True)
            o = _dot(pd.astype(bf), v_s[h, lo:hi_, :])
            if i:
                po = jnp.exp2(so - m)
                l = l + jnp.sum(po, axis=1, keepdims=True)
                o = o + _dot(po.astype(bf), v_s[h, :lo, :])
            ctx_s[h, lo:hi_, :] = (o * (1.0 / l)).astype(bf)
        return carry
    jax.lax.fori_loop(0, G, head, 0)

    def outp(i, carry):
        r = pl.multiple_of(i * 512, 512)
        cb = jnp.concatenate([ctx_s[h, pl.ds(r, 512), :] for h in range(G)], axis=1)
        t = _dot(cb, wo_ref[...])

        @pl.when(g == 0)
        def _():
            acc_s[pl.ds(r, 512), :] = t

        @pl.when(g > 0)
        def _():
            acc_s[pl.ds(r, 512), :] += t

        @pl.when(g == ng - 1)
        def _():
            xb = x_ref[pl.ds(r, 512), :]
            z = jnp.sum((xb * gw_ref[...]).astype(jnp.float32), axis=1, keepdims=True)
            gt = jax.nn.sigmoid(z)
            res = gt * a_out[pl.ds(r, 512), :] + (1.0 - gt) * acc_s[pl.ds(r, 512), :]
            o_ref[pl.ds(r, 512), :] = res.astype(o_ref.dtype)
        return carry
    jax.lax.fori_loop(0, S // 512, outp, 0)


@jax.jit
def pallas_gated_mix__sliding_local_dilated__compressed_kv_cla__prompt_kernel(
    A_x, A_wqkv, A_wo, B_x, B_c_kv, B_w_q, B_w_uk, B_w_uv, B_w_o, gate_w,
):
    del B_x
    _, S, M = A_x.shape
    C = B_c_kv.shape[-1]
    H, D = B_w_q.shape[1:]
    full = lambda shape: pl.BlockSpec(shape, lambda g: (0,) * len(shape))
    f32, bf = jnp.float32, jnp.bfloat16
    out = pl.pallas_call(
        functools.partial(_kernel, HA=32, W=8, DIL=2),
        grid=(H // G,),
        in_specs=[
            full((S, M)), full((M, 3 * M)), full((M, M)), full((S, C)),
            pl.BlockSpec((M, G * D), lambda g: (0, g)),
            pl.BlockSpec((C, G * D), lambda g: (0, g)),
            pl.BlockSpec((C, G * D), lambda g: (0, g)),
            pl.BlockSpec((G * D, M), lambda g: (g, 0)),
            full((1, M)),
        ],
        out_specs=full((S, M)),
        out_shape=jax.ShapeDtypeStruct((S, M), A_x.dtype),
        scratch_shapes=[pltpu.VMEM((G, S, D), bf)] * 4 + [
            pltpu.VMEM((S, M), f32), pltpu.VMEM((3, S + 16, M), f32), pltpu.VMEM((S, M), f32),
            pltpu.VMEM((3, M, M), bf)],
        compiler_params=pltpu.CompilerParams(
            dimension_semantics=("arbitrary",), vmem_limit_bytes=110 * 1024 * 1024),
    )(A_x.reshape(S, M), A_wqkv, A_wo, B_c_kv.reshape(S, C),
      B_w_q.reshape(M, H * D), B_w_uk.reshape(C, H * D), B_w_uv.reshape(C, H * D),
      B_w_o.reshape(H * D, M), gate_w.reshape(1, M))
    return out.reshape(1, S, M)
```

```python
import functools

import jax
import jax.numpy as jnp
import numpy as np
import jax.experimental.pallas as pl
import jax.experimental.pallas.tpu as pltpu

LOG2E = 1.4426950408889634
NT = (((1,), (1,)), ((), ()))
G = 8
BQ = 256
BA = 256


def _dot(a, b):
    return jnp.dot(a, b, preferred_element_type=jnp.float32)


def _nt(a, b):
    return jax.lax.dot_general(a, b, NT, preferred_element_type=jnp.float32)


def _kernel(xt_ref, wqkv_ref, woa_ref, c_ref, wq_ref, wk_ref, wv_ref, wo_ref, gw_ref,
            o_ref, q_s, k_s, v_s, ctx_s, acc_s, a_qkv, a_out, w3, x_ref, woat, wq_s, wk_s, wv_s, *, HA, W, DIL):
    g = pl.program_id(0)
    ng = pl.num_programs(0)
    S, M = x_ref.shape
    D = q_s.shape[-1]
    DH = M // HA
    bf = jnp.bfloat16
    PAD = a_qkv.shape[1] - S

    @pl.when(g == 0)
    def _():
        a_qkv[:, :PAD, :] = jnp.zeros((3, PAD, M), jnp.float32)

        for t in range(3):
            w3[t] = wqkv_ref[:, t * M:(t + 1) * M]

        x_ref[...] = xt_ref[...].T
        woat[...] = woa_ref[...].T

        def proj(i, carry):
            r = pl.multiple_of(i * BA, BA)
            xb = x_ref[pl.ds(r, BA), :]
            for t in range(3):
                a_qkv[t, pl.ds(PAD + r, BA), :] = _dot(xb, w3[t]).astype(bf).astype(jnp.float32)
            return carry
        jax.lax.fori_loop(0, S // BA, proj, 0)

        li = jax.lax.broadcasted_iota(jnp.int32, (M, 128), 0)
        hi = jax.lax.broadcasted_iota(jnp.int32, (M, 128), 1)
        seg = ((li >= hi * DH) & (li < hi * DH + DH)).astype(bf)
        li = jax.lax.broadcasted_iota(jnp.int32, (128, M), 1)
        hi = jax.lax.broadcasted_iota(jnp.int32, (128, M), 0)
        segt = ((li >= hi * DH) & (li < hi * DH + DH)).astype(bf)

        def loc(i, carry):
            r = pl.multiple_of(i * BA, BA)
            q = a_qkv[0, pl.ds(PAD + r, BA), :]
            pos = r + jax.lax.broadcasted_iota(jnp.int32, (BA, 128), 0)
            ls = []
            kk = a_qkv[1, pl.ds(r, BA + PAD), :]
            vv = a_qkv[2, pl.ds(r, BA + PAD), :]
            for w in range(W):
                kw = kk[PAD - w * DIL:PAD - w * DIL + BA]
                l = _dot((q * kw).astype(bf), seg) * (DH ** -0.5)
                if w:
                    l = jnp.where(pos >= w * DIL, l, -1e9)
                ls.append(l)
            m = functools.reduce(jnp.maximum, ls)
            es = [jnp.exp(l - m) for l in ls]
            inv = 1.0 / functools.reduce(jnp.add, es)
            o = None
            for w in range(W):
                vw = vv[PAD - w * DIL:PAD - w * DIL + BA]
                t = _dot((es[w] * inv).astype(bf), segt) * vw
                o = t if o is None else o + t
            a_out[:, pl.ds(r, BA)] = _nt(woat[...], o.astype(bf))
            return carry
        jax.lax.fori_loop(0, S // BA, loc, 0)

    for src, dst in ((wq_ref, wq_s), (wk_ref, wk_s), (wv_ref, wv_s)):
        for h in range(G):
            dst[:, h * D:(h + 1) * D] = src[:, h, :]

    def proj_b(i, carry):
        r = pl.multiple_of(i * 512, 512)
        q = _dot(x_ref[pl.ds(r, 512), :], wq_s[...]) * (D ** -0.5 * LOG2E)
        cb = c_ref[pl.ds(r, 512), :]
        k = _dot(cb, wk_s[...])
        v = _dot(cb, wv_s[...])
        for h in range(G):
            q_s[h, pl.ds(r, 512), :] = q[:, h * D:(h + 1) * D].astype(bf)
            k_s[h, pl.ds(r, 512), :] = k[:, h * D:(h + 1) * D].astype(bf)
            v_s[h, pl.ds(r, 512), :] = v[:, h * D:(h + 1) * D].astype(bf)
        return carry
    jax.lax.fori_loop(0, S // 512, proj_b, 0)

    def head(h, carry):
        row = jax.lax.broadcasted_iota(jnp.int32, (BQ, BQ), 0)
        col = jax.lax.broadcasted_iota(jnp.int32, (BQ, BQ), 1)
        for i in range(S // BQ):
            lo, hi_ = i * BQ, (i + 1) * BQ
            q = q_s[h, lo:hi_, :]
            sd = jax.lax.dot_general(q, k_s[h, lo:hi_, :], NT, preferred_element_type=jnp.float32)
            sd = jnp.where(col <= row, sd, -1e9 * LOG2E)
            m = jnp.max(sd, axis=1, keepdims=True)
            if i:
                so = jax.lax.dot_general(q, k_s[h, :lo, :], NT, preferred_element_type=jnp.float32)
                m = jnp.maximum(m, jnp.max(so, axis=1, keepdims=True))
            pd = jnp.exp2(sd - m)
            l = jnp.sum(pd, axis=1, keepdims=True)
            o = _dot(pd.astype(bf), v_s[h, lo:hi_, :])
            if i:
                po = jnp.exp2(so - m)
                l = l + jnp.sum(po, axis=1, keepdims=True)
                o = o + _dot(po.astype(bf), v_s[h, :lo, :])
            ctx_s[h, lo:hi_, :] = (o * (1.0 / l)).astype(bf)
        return carry
    jax.lax.fori_loop(0, G, head, 0)

    def outp(i, carry):
        r = pl.multiple_of(i * 512, 512)
        cb = jnp.concatenate([ctx_s[h, pl.ds(r, 512), :] for h in range(G)], axis=1)
        wo = jnp.concatenate([wo_ref[h] for h in range(G)], axis=1)
        t = _nt(wo, cb)

        @pl.when(g == 0)
        def _():
            acc_s[:, pl.ds(r, 512)] = t

        @pl.when((g > 0) & (g < ng - 1))
        def _():
            acc_s[:, pl.ds(r, 512)] += t

        @pl.when(g == ng - 1)
        def _():
            z = _dot(jnp.broadcast_to(gw_ref[...], (16, M)), xt_ref[:, pl.ds(r, 512)])[:1]
            gt = jax.nn.sigmoid(z)
            res = gt * a_out[:, pl.ds(r, 512)] + (1.0 - gt) * (acc_s[:, pl.ds(r, 512)] + t)
            o_ref[:, pl.ds(r, 512)] = res.astype(o_ref.dtype)
        return carry
    jax.lax.fori_loop(0, S // 512, outp, 0)


@jax.jit
def pallas_gated_mix__sliding_local_dilated__compressed_kv_cla__prompt_kernel(
    A_x, A_wqkv, A_wo, B_x, B_c_kv, B_w_q, B_w_uk, B_w_uv, B_w_o, gate_w,
):
    del B_x
    _, S, M = A_x.shape
    C = B_c_kv.shape[-1]
    H, D = B_w_q.shape[1:]
    full = lambda shape: pl.BlockSpec(shape, lambda g: (0,) * len(shape))
    f32, bf = jnp.float32, jnp.bfloat16
    out = pl.pallas_call(
        functools.partial(_kernel, HA=32, W=8, DIL=2),
        grid=(H // G,),
        in_specs=[
            full((M, S)), full((M, 3 * M)), full((M, M)), full((S, C)),
            pl.BlockSpec((M, G, D), lambda g: (0, g, 0)),
            pl.BlockSpec((C, G, D), lambda g: (0, g, 0)),
            pl.BlockSpec((C, G, D), lambda g: (0, g, 0)),
            pl.BlockSpec((G, M, D), lambda g: (g, 0, 0)),
            full((1, M)),
        ],
        out_specs=full((M, S)),
        out_shape=jax.ShapeDtypeStruct((M, S), A_x.dtype),
        scratch_shapes=[pltpu.VMEM((G, S, D), bf)] * 4 + [
            pltpu.VMEM((M, S), f32), pltpu.VMEM((3, S + 16, M), f32), pltpu.VMEM((M, S), f32),
            pltpu.VMEM((3, M, M), bf), pltpu.VMEM((S, M), bf), pltpu.VMEM((M, M), bf),
            pltpu.VMEM((M, G * D), bf), pltpu.VMEM((C, G * D), bf), pltpu.VMEM((C, G * D), bf)],
        compiler_params=pltpu.CompilerParams(
            dimension_semantics=("arbitrary",), vmem_limit_bytes=110 * 1024 * 1024),
    )(A_x.reshape(S, M).T, A_wqkv, A_wo, B_c_kv.reshape(S, C),
      B_w_q, B_w_uk, B_w_uv,
      B_w_o.transpose(0, 2, 1), gate_w.reshape(1, M))
    return out.T.reshape(1, S, M)
```

```python
import functools

import jax
import jax.numpy as jnp
import numpy as np
import jax.experimental.pallas as pl
import jax.experimental.pallas.tpu as pltpu

LOG2E = 1.4426950408889634
NT = (((1,), (1,)), ((), ()))
G = 8
BP = 512
BQ = 512
KB = 128
BA = 512
BR = 1024
HN = 4


def _dot(a, b):
    return jnp.dot(a, b, preferred_element_type=jnp.float32)


def _nt(a, b):
    return jax.lax.dot_general(a, b, NT, preferred_element_type=jnp.float32)


def _kernel(xt_ref, wqkv_ref, woa_ref, c_ref, wq_ref, wk_ref, wv_ref, wo_ref, gw_ref,
            o_ref, q_s, k_s, v_s, ctx_s, acc_s, a_qkv, a_out, w3, x_ref, woat, wq_s, wk_s, wv_s, rq, rk, rv, sems, *, HA, W, DIL):
    g = pl.program_id(0)
    ng = pl.num_programs(0)
    S, M = x_ref.shape
    D = q_s.shape[-1]
    DH = M // HA
    bf = jnp.bfloat16
    PAD = a_qkv.shape[1] - S

    @pl.when(g == 0)
    def _():
        cps = [pltpu.make_async_copy(a, b, sems.at[n]) for n, (a, b) in
               enumerate(((wq_ref, rq), (wk_ref, rk), (wv_ref, rv)))]
        for cp in cps:
            cp.start()
        a_qkv[:, :PAD, :] = jnp.zeros((3, PAD, M), jnp.float32)

        for t in range(3):
            w3[t] = wqkv_ref[:, t * M:(t + 1) * M]

        x_ref[...] = xt_ref[...].T
        woat[...] = woa_ref[...].T

        def proj(i, carry):
            r = pl.multiple_of(i * BA, BA)
            xb = x_ref[pl.ds(r, BA), :]
            for t in range(3):
                a_qkv[t, pl.ds(PAD + r, BA), :] = _dot(xb, w3[t]).astype(bf).astype(jnp.float32)
            return carry
        jax.lax.fori_loop(0, S // BA, proj, 0)

        li = jax.lax.broadcasted_iota(jnp.int32, (M, 128), 0)
        hi = jax.lax.broadcasted_iota(jnp.int32, (M, 128), 1)
        seg = ((li >= hi * DH) & (li < hi * DH + DH)).astype(bf)
        li = jax.lax.broadcasted_iota(jnp.int32, (128, M), 1)
        hi = jax.lax.broadcasted_iota(jnp.int32, (128, M), 0)
        segt = ((li >= hi * DH) & (li < hi * DH + DH)).astype(bf)

        def loc(i, carry):
            r = pl.multiple_of(i * BA, BA)
            q = a_qkv[0, pl.ds(PAD + r, BA), :]
            pos = r + jax.lax.broadcasted_iota(jnp.int32, (BA, 128), 0)
            ls = []
            kk = a_qkv[1, pl.ds(r, BA + PAD), :]
            vv = a_qkv[2, pl.ds(r, BA + PAD), :]
            for w in range(W):
                kw = kk[PAD - w * DIL:PAD - w * DIL + BA]
                l = _dot((q * kw).astype(bf), seg) * (DH ** -0.5)
                if w:
                    l = jnp.where(pos >= w * DIL, l, -1e9)
                ls.append(l)
            m = functools.reduce(jnp.maximum, ls)
            es = [jnp.exp(l - m) for l in ls]
            inv = 1.0 / functools.reduce(jnp.add, es)
            o = None
            for w in range(W):
                vw = vv[PAD - w * DIL:PAD - w * DIL + BA]
                t = _dot((es[w] * inv).astype(bf), segt) * vw
                o = t if o is None else o + t
            a_out[:, pl.ds(r, BA)] = _nt(woat[...], o.astype(bf))
            return carry
        jax.lax.fori_loop(0, S // BA, loc, 0)
        for cp in cps:
            cp.wait()

    def unpack(pairs, gg):
        def body(i, carry):
            r = pl.multiple_of(i * 64, 64)
            for src, dst in pairs:
                st, hp = src.shape[0] // dst.shape[0] // 2, G // 2
                blk = src.at[pl.ds(pl.multiple_of(i * (128 * st), 128 * st), 128 * st), :]
                for j in range(hp):
                    u = blk.bitcast(jnp.uint32)[pl.ds(gg * hp + j, 64, stride=st), :]
                    lo = pltpu.bitcast(u << 16, jnp.float32)
                    hi = pltpu.bitcast(u & np.uint32(0xFFFF0000), jnp.float32)
                    dst[pl.ds(r, 64), 2 * j * D:(2 * j + 1) * D] = lo.astype(bf)
                    dst[pl.ds(r, 64), (2 * j + 1) * D:(2 * j + 2) * D] = hi.astype(bf)
            return carry
        jax.lax.fori_loop(0, pairs[0][1].shape[0] // 64, body, 0)

    for gg in range(rq.shape[0] // M // G):
        @pl.when(g == gg)
        def _(gg=gg):
            unpack(((rq, wq_s),), gg)
            unpack(((rk, wk_s), (rv, wv_s)), gg)

    def proj_b(i, carry):
        r = pl.multiple_of((i // (G // HN)) * BR, BR)
        h0 = (i % (G // HN)) * HN
        cs = pl.ds(pl.multiple_of(h0 * D, HN * D), HN * D)
        q = _dot(x_ref[pl.ds(r, BR), :], wq_s[:, cs]) * (D ** -0.5 * LOG2E)
        cb = c_ref[pl.ds(r, BR), :]
        k = _dot(cb, wk_s[:, cs])
        v = _dot(cb, wv_s[:, cs])
        for h in range(HN):
            q_s[h0 + h, pl.ds(r, BR), :] = q[:, h * D:(h + 1) * D].astype(bf)
            k_s[h0 + h, pl.ds(r, BR), :] = k[:, h * D:(h + 1) * D].astype(bf)
            v_s[h0 + h, pl.ds(r, BR), :] = v[:, h * D:(h + 1) * D].astype(bf)
        return carry
    jax.lax.fori_loop(0, S // BR * (G // HN), proj_b, 0)

    def head(h, carry):
        row = jax.lax.broadcasted_iota(jnp.int32, (KB, KB), 0)
        col = jax.lax.broadcasted_iota(jnp.int32, (KB, KB), 1)
        nb = BQ // KB
        for i in range(S // BQ):
            lo, hi_ = i * BQ, (i + 1) * BQ
            sd = []
            for j in range(nb):
                k0 = lo + j * KB
                t = _nt(q_s[h, k0:hi_, :], k_s[h, k0:k0 + KB, :])
                top = jnp.where(col <= row, t[:KB], -1e9 * LOG2E)
                sd.append(jnp.concatenate([top, t[KB:]], axis=0) if j < nb - 1 else top)
            rows = lambda xs, f, r: functools.reduce(
                f, [xs[j][(r - j) * KB:(r - j + 1) * KB] for j in range(r + 1)])
            stack = lambda xs, f: jnp.concatenate([rows(xs, f, r) for r in range(nb)], axis=0)
            m = jnp.max(stack(sd, jnp.maximum), axis=1, keepdims=True)
            if i:
                so = _nt(q_s[h, lo:hi_, :], k_s[h, :lo, :])
                m = jnp.maximum(m, jnp.max(so, axis=1, keepdims=True))
            pd = [jnp.exp2(sd[j] - m[j * KB:]) for j in range(nb)]
            l = jnp.sum(stack(pd, jnp.add), axis=1, keepdims=True)
            o = stack([_dot(pd[j].astype(bf), v_s[h, lo + j * KB:lo + (j + 1) * KB, :])
                       for j in range(nb)], jnp.add)
            if i:
                po = jnp.exp2(so - m)
                l = l + jnp.sum(po, axis=1, keepdims=True)
                o = o + _dot(po.astype(bf), v_s[h, :lo, :])
            ctx_s[h, lo:hi_, :] = (o * (1.0 / l)).astype(bf)
        return carry
    jax.lax.fori_loop(0, G, head, 0)

    def outp(i, carry):
        r = pl.multiple_of(i * BP, BP)
        cb = jnp.concatenate([ctx_s[h, pl.ds(r, BP), :] for h in range(G)], axis=1)
        wo = jnp.concatenate([wo_ref[h] for h in range(G)], axis=1)
        t = _nt(wo, cb)

        @pl.when(g == 0)
        def _():
            acc_s[:, pl.ds(r, BP)] = t

        @pl.when((g > 0) & (g < ng - 1))
        def _():
            acc_s[:, pl.ds(r, BP)] += t

        @pl.when(g == ng - 1)
        def _():
            z = _dot(jnp.broadcast_to(gw_ref[...], (16, M)), xt_ref[:, pl.ds(r, BP)])[:1]
            gt = jax.nn.sigmoid(z)
            res = gt * a_out[:, pl.ds(r, BP)] + (1.0 - gt) * (acc_s[:, pl.ds(r, BP)] + t)
            o_ref[:, pl.ds(r, BP)] = res.astype(o_ref.dtype)
        return carry
    jax.lax.fori_loop(0, S // BP, outp, 0)


@jax.jit
def pallas_gated_mix__sliding_local_dilated__compressed_kv_cla__prompt_kernel(
    A_x, A_wqkv, A_wo, B_x, B_c_kv, B_w_q, B_w_uk, B_w_uv, B_w_o, gate_w,
):
    del B_x
    _, S, M = A_x.shape
    C = B_c_kv.shape[-1]
    H, D = B_w_q.shape[1:]
    full = lambda shape: pl.BlockSpec(shape, lambda g: (0,) * len(shape))
    f32, bf = jnp.float32, jnp.bfloat16
    out = pl.pallas_call(
        functools.partial(_kernel, HA=32, W=8, DIL=2),
        grid=(H // G,),
        in_specs=[
            full((M, S)), full((M, 3 * M)), full((M, M)), full((S, C)),
            pl.BlockSpec(memory_space=pl.ANY),
            pl.BlockSpec(memory_space=pl.ANY),
            pl.BlockSpec(memory_space=pl.ANY),
            pl.BlockSpec((G, M, D), lambda g: (g, 0, 0)),
            full((1, M)),
        ],
        out_specs=full((M, S)),
        out_shape=jax.ShapeDtypeStruct((M, S), A_x.dtype),
        scratch_shapes=[pltpu.VMEM((G, S, D), bf)] * 4 + [
            pltpu.VMEM((M, S), f32), pltpu.VMEM((3, S + 16, M), f32), pltpu.VMEM((M, S), f32),
            pltpu.VMEM((3, M, M), bf), pltpu.VMEM((S, M), bf), pltpu.VMEM((M, M), bf),
            pltpu.VMEM((M, G * D), bf), pltpu.VMEM((C, G * D), bf), pltpu.VMEM((C, G * D), bf),
            pltpu.VMEM((M * H, D), bf), pltpu.VMEM((C * H, D), bf), pltpu.VMEM((C * H, D), bf),
            pltpu.SemaphoreType.DMA((3,))],
        compiler_params=pltpu.CompilerParams(
            dimension_semantics=("arbitrary",), vmem_limit_bytes=110 * 1024 * 1024),
    )(A_x.reshape(S, M).T, A_wqkv, A_wo, B_c_kv.reshape(S, C),
      B_w_q.reshape(M * H, D), B_w_uk.reshape(C * H, D), B_w_uv.reshape(C * H, D),
      B_w_o.transpose(0, 2, 1), gate_w.reshape(1, M))
    return out.T.reshape(1, S, M)
```
